```python
import os as _os
_os.environ.setdefault("JAX_PLATFORMS", "cpu")
import jax
import jax.numpy as jnp

def _softmax(x, axis=-1):
    return jax.nn.softmax(x, axis=axis)
def _gelu(x):
    return jax.nn.gelu(x, approximate=True)
def _silu(x):
    return jax.nn.silu(x)
def _sigmoid(x):
    return jax.nn.sigmoid(x)
def _layernorm(x, axis=-1, eps=1e-5):
    m = jnp.mean(x, axis=axis, keepdims=True)
    v = jnp.var(x, axis=axis, keepdims=True)
    return (x - m) / jnp.sqrt(v + eps)
def _scatter_add(tgt, idx, src, axis=0):
    return tgt.at[idx].add(src)
def _segment_sum(src, seg, n):
    return jax.ops.segment_sum(src, seg, n)
class _Rng:
    def __init__(self, key):
        self._k = key
    def _next(self):
        self._k, sub = jax.random.split(self._k)
        return sub
    def normal(self, shape):
        return jax.random.normal(self._next(), shape, dtype=jnp.bfloat16)
    def randint(self, lo, hi, shape):
        return jax.random.randint(self._next(), shape, lo, hi, dtype=jnp.int32)
    def uniform(self, shape, lo=0.0, hi=1.0):
        return jax.random.uniform(self._next(), shape, jnp.bfloat16, lo, hi)
    def permutation(self, n):
        return jax.random.permutation(self._next(), n)


kernel_name = 'parallel_sum__sliding_block__moe_arch_mod__prompt'

def setup_inputs():
    _rng = _Rng(jax.random.key(int.from_bytes(__import__("os").urandom(4), "little")))
    _w = (lambda a: (lambda t: t.astype(jnp.bfloat16) if jnp.issubdtype(t.dtype, jnp.floating) else t)(jnp.asarray(a)))
    def _A_setup():
        B, S, D = 1, 2048, 512
        return {
            "x": _w((lambda *s: _rng.normal(s) * 0.05)(B, S, D)),
            "wqkv": _w((lambda *s: _rng.normal(s) * 0.05)(D, 3 * D)),
            "wo": _w((lambda *s: _rng.normal(s) * 0.05)(D, D)),
        }
    _A_in = _A_setup()

    def _B_setup():
        B, S, D, F, C = 1, 2048, 512, 1376, 1
        return {
            "x": _w((lambda *s: _rng.normal(s) * 0.05)(B, S, D)),
            "w_r": _w((lambda *s: _rng.normal(s) * 0.05)(D)),
            "w_gate": _w((lambda *s: _rng.normal(s) * 0.05)(D, F)),
            "w_up": _w((lambda *s: _rng.normal(s) * 0.05)(D, F)),
            "w_down": _w((lambda *s: _rng.normal(s) * 0.05)(F, D)),
        }
    _B_in = _B_setup()

    return {
        "A_x": _A_in["x"],
        "A_wqkv": _A_in["wqkv"],
        "A_wo": _A_in["wo"],
        "B_x": _B_in["x"],
        "B_w_r": _B_in["w_r"],
        "B_w_gate": _B_in["w_gate"],
        "B_w_up": _B_in["w_up"],
        "B_w_down": _B_in["w_down"],
    }

def reference(A_x, A_wqkv, A_wo, B_x, B_w_r, B_w_gate, B_w_up, B_w_down):
    def _A_ref(x, wqkv, wo):
        B, S, D = x.shape
        H = 32; Dh = D // H; W = 256
        qkv = (lambda x, *d: x.transpose(*d))((x @ wqkv).reshape(B, S, 3, H, Dh), 2, 0, 3, 1, 4)
        q, k, v = qkv[0], qkv[1], qkv[2]
        scores = jnp.einsum("bhqd,bhkd->bhqk", q, k) * (Dh ** -0.5)
        idx = jnp.arange(S)
        mask = (idx[:, None] - idx[None, :] >= 0) & (idx[:, None] - idx[None, :] < W)
        scores = jnp.where(mask[None, None], scores, -1e9)
        p = _softmax(scores, axis=-1)
        o = jnp.einsum("bhqk,bhkd->bhqd", p, v)
        return (lambda x, *d: x.transpose(*d))(o, 0, 2, 1, 3).reshape(B, S, D) @ wo

    def _B_ref(x, w_r, w_gate, w_up, w_down):
        B, S, D = x.shape
        C = 1
        r = x @ w_r
        idx = jnp.argsort(-r, axis=-1)[:, :C]
        idx_e = jnp.repeat(idx.reshape(B, C, 1), D, axis=2)
        x_sel = jnp.take_along_axis(x, idx_e, axis=1)
        g = _silu(x_sel @ w_gate)
        u = x_sel @ w_up
        y = (g * u) @ w_down
        r_sel = _sigmoid(jnp.take_along_axis(r, idx, axis=1))
        y = y * r_sel.reshape(B, C, 1)
        b_off = (jnp.arange(B) * S).reshape(B, 1)
        flat_idx = (idx + b_off).reshape(B * C)
        zero = (x * 0.0).reshape(B * S, D)
        upd = _scatter_add(zero, flat_idx, y.reshape(B * C, D), axis=0)
        return x + upd.reshape(B, S, D)

    x = A_x
    xn = _layernorm(x, axis=-1)
    return x + _A_ref(xn, A_wqkv, A_wo) + _B_ref(xn, B_w_r, B_w_gate, B_w_up, B_w_down)
```

```python
import functools
import math

import jax
import jax.numpy as jnp
from jax import lax
import jax.experimental.pallas as pl
import jax.experimental.pallas.tpu as pltpu

S = 2048
D = 512
H = 32
DH = 16
W = 256
F = 1376
TQ = 128
NT_ = S // TQ
EPS = 1e-5
NEG = -1e9
LOG2E = math.log2(math.e)
QSCALE = (DH ** -0.5) * LOG2E
NT = (((1,), (1,)), ((), ()))
f32 = jnp.float32
bf16 = jnp.bfloat16
u32 = jnp.uint32


def _unpack(u, i):
    return pltpu.unpack_elementwise(u, index=i, packed_dtype=bf16, unpacked_dtype=f32)


def _ipack(a, b):
    return pltpu.pack_elementwise([a, b], packed_dtype=bf16)


def make_kernel(cfg):
    LB = cfg.get("lb", 9)
    LW = cfg.get("lw", 4)

    def kernel(x_hbm, wqkv_hbm, wo_hbm, wr_hbm, wg_hbm, wu_hbm, wd_hbm, out_hbm,
               x_v, wqkv_v, wo_v, wr_v, wg_v, wu_v, wd_v,
               wvt_v, wo_u, q_u, k_u, vt_u, xn_u, res_v, ot_v, out_v, cm_v,
               sem_x, sem_w, sem_o):
        def xcopy(j):
            return pltpu.make_async_copy(x_hbm.at[0, pl.ds(j * TQ, TQ), :], x_v.at[pl.ds(j * TQ, TQ), :], sem_x.at[j])
        cp_wqkv = pltpu.make_async_copy(wqkv_hbm, wqkv_v, sem_w.at[0])
        cp_wr = pltpu.make_async_copy(wr_hbm, wr_v, sem_w.at[1])
        cp_wo = pltpu.make_async_copy(wo_hbm, wo_v, sem_w.at[2])
        cp_wg = pltpu.make_async_copy(wg_hbm, wg_v, sem_w.at[3])
        cp_wu = pltpu.make_async_copy(wu_hbm, wu_v, sem_w.at[4])
        cp_wd = pltpu.make_async_copy(wd_hbm, wd_v, sem_w.at[5])
        xcopy(0).start()
        cp_wr.start()
        cp_wqkv.start()
        for j in range(1, NT_):
            xcopy(j).start()
        cp_wo.start()
        cp_wg.start()
        cp_wu.start()
        cp_wd.start()

        lane8 = lax.broadcasted_iota(jnp.int32, (8, 128), 1)
        for h in range(8):
            cm_v[h] = jnp.where(lane8 // DH == h, u32(0xFFFFFFFF), u32(0))
        lo8 = lane8 < 64
        lane_1 = lax.broadcasted_iota(jnp.int32, (1, 128), 1)
        lane_f = lax.broadcasted_iota(jnp.int32, (16, 128), 1)
        odd_blk = (lane_f // 32) % 2 == 1
        lane32 = lax.broadcasted_iota(jnp.int32, (32, 128), 1)
        row32 = lax.broadcasted_iota(jnp.int32, (32, 128), 0)
        m_old = row32 > (lane32 % 32)

        cp_wr.wait()
        cp_wqkv.wait()

        def prep_wv():
            wv = wqkv_v[:, 2 * D:3 * D]
            wvt = wv.astype(f32).T.astype(bf16)
            u = pltpu.bitcast(wvt, u32)
            e = _unpack(u, 0).reshape(H, 8, D)
            o = _unpack(u, 1).reshape(H, 8, D)
            wpi = jnp.concatenate([e, o], axis=1).reshape(D, D).astype(bf16)
            wvt_v[pl.ds(0, D), :] = wpi
            wr = wr_v[...].reshape(1, D)
            wvt_v[pl.ds(D, 16), :] = jnp.broadcast_to(wr, (16, D))

        def prep_wo():
            cp_wo.wait()
            wo_u[...] = pltpu.bitcast(wo_v[...], u32)

        state = {}

        def layer_norm(j):
            xcopy(j).wait()
            xt = x_v[pl.ds(j * TQ, TQ), :]
            u = pltpu.bitcast(xt, u32)
            halves = []
            for i in range(2):
                xf = _unpack(u, i)
                mean = jnp.mean(xf, axis=-1, keepdims=True)
                xc = xf - mean
                var = jnp.mean(xc * xc, axis=-1, keepdims=True)
                m_b = mean.astype(bf16).astype(f32)
                d_b = (xf - m_b).astype(bf16).astype(f32)
                v_b = (var.astype(bf16) + jnp.asarray(EPS, bf16)).astype(f32)
                sd = jnp.sqrt(v_b).astype(bf16).astype(f32)
                halves.append(d_b / sd)
            xe, xo = halves
            xn_pi = jnp.concatenate([xe, xo], axis=0).astype(bf16)
            un = _ipack(xe, xo)
            xn_u[pl.ds(j * 64, 64), :] = un
            xn_nat = pltpu.bitcast(un, bf16).astype(f32)
            x3 = xn_nat.reshape(8, 16, D)
            xn_sig = pltpu.bitcast(_ipack(x3[:, 0:8, :], x3[:, 8:16, :]).reshape(64, D), bf16)
            res_v[pl.ds(j * TQ, TQ), :] = xt.astype(f32) + xn_nat
            state["xn", j] = (xn_pi, xn_sig)

        def proj_qk(j):
            xn_pi, _ = state["xn", j]
            for part in range(2):
                for g in range(4):
                    c0 = part * D + g * 128
                    r = jnp.dot(xn_pi, wqkv_v[:, c0:c0 + 128], preferred_element_type=f32)
                    if part == 0:
                        r = r * QSCALE
                    pk = _ipack(r[0:64], r[64:128])
                    dst = q_u if part == 0 else k_u
                    dst[g, pl.ds(j * 64, 64), :] = pk

        def proj_vt(j):
            _, xn_sig = state.pop(("xn", j))
            r = lax.dot_general(wvt_v[...], xn_sig, NT, preferred_element_type=f32)
            v3 = r[0:D].reshape(H, 16, 128)
            vt_u[:, pl.ds(j * TQ, TQ)] = _ipack(v3[:, 0:8, :], v3[:, 8:16, :]).reshape(D // 2, 128)
            rr = r[D:D + 8]
            if j == 0:
                state["rmax"] = rr
                state["ridx"] = jnp.zeros((8, 128), jnp.int32)
            else:
                better = rr > state["rmax"]
                state["rmax"] = jnp.where(better, rr, state["rmax"])
                state["ridx"] = jnp.where(better, j, state["ridx"])

        def ffn():
            rmax, rj = state["rmax"], state["ridx"]
            l16 = lane8 % 16
            tok_in = (lane8 // 16) * 16 + (l16 // 2) + 8 * (l16 % 2)
            tok = rj * TQ + tok_in
            best = jnp.max(rmax, axis=1, keepdims=True)
            idx = jnp.min(jnp.where(rmax == best, tok, S))
            idx = jnp.clip(idx, 0, S - 1)
            blk = idx // 16
            cp_wg.wait(); cp_wu.wait(); cp_wd.wait()
            xb = pltpu.bitcast(xn_u[pl.ds(pl.multiple_of(blk * 8, 8), 8), :], bf16)
            g = jnp.dot(xb, wg_v[...], preferred_element_type=f32).astype(bf16).astype(f32)
            up = jnp.dot(xb, wu_v[...], preferred_element_type=f32).astype(bf16).astype(f32)
            act = (g * jax.nn.sigmoid(g)).astype(bf16).astype(f32)
            hh = (act * up).astype(bf16)
            y = jnp.dot(hh, wd_v[...], preferred_element_type=f32).astype(bf16).astype(f32)
            gate = jax.nn.sigmoid(best[0:1].astype(bf16).astype(f32)).astype(bf16).astype(f32)
            rows = lax.broadcasted_iota(jnp.int32, (16, D), 0)
            upd = jnp.where(rows == idx % 16, (y * gate).astype(bf16).astype(f32), 0.0)
            sl = pl.ds(pl.multiple_of(blk * 16, 16), 16)
            res_v[sl, :] = res_v[sl, :] + upd

        def unit_info(u):
            b, r = divmod(u, 4)
            j, c = divmod(b, 8)
            par, t = divmod(r, 2)
            return j, c, par, t

        def qk(u):
            j, c, par, t = unit_info(u)
            g, half = c // 2, c % 2
            s = 4 * j + 2 * par + t
            lo = max(0, 32 * s - W)
            hi = 32 * s + 32
            qt = q_u[g, pl.ds(16 * s, 16), :]
            parts = []
            for p in range(4):
                mk = cm_v[4 * half + (p + 2 * t) % 4]
                parts.append(qt & jnp.concatenate([mk, mk], 0))
            b = pltpu.bitcast(jnp.concatenate(parts, axis=0), bf16)
            kk = pltpu.bitcast(k_u[g, pl.ds(lo // 2, (hi - lo) // 2), :], bf16)
            state["s", u] = lax.dot_general(kk, b, NT, preferred_element_type=f32)

        def softmax(u):
            j, c, par, t = unit_info(u)
            s = 4 * j + 2 * par + t
            st = state.pop(("s", u))
            n = st.shape[0]
            lo = max(0, 32 * s - W)
            has_old = 32 * s - W >= 0
            pieces = []
            a = 0
            if has_old:
                pieces.append(jnp.where(m_old, st[0:32], NEG))
                a = 32
            if n - 32 > a:
                pieces.append(st[a:n - 32])
            pieces.append(jnp.where(m_old, NEG, st[n - 32:n]))
            st = jnp.concatenate(pieces, axis=0) if len(pieces) > 1 else pieces[0]
            mx = jnp.max(st, axis=0, keepdims=True)
            p = jnp.exp2(st - mx)
            l = jnp.sum(p, axis=0, keepdims=True)
            p3 = p.reshape(n // 16, 16, 128)
            uu = _ipack(p3[:, 0:8, :], p3[:, 8:16, :])
            state["p", u] = ([uu[r] for r in range(n // 16)], l)

        def exchange(u0):
            j, c, par, _ = unit_info(u0)
            jb = max(0, j - 2)
            nblk = 8 * (j - jb + 1)
            (p1, l1), (p2, l2) = state.pop(("p", u0)), state.pop(("p", u0 + 1))
            z = jnp.zeros((8, 128), u32)
            s0 = 4 * j + 2 * par
            off1 = (max(0, 32 * s0 - W) - 128 * jb) // 16
            off2 = (max(0, 32 * (s0 + 1) - W) - 128 * jb) // 16
            a = [z] * off1 + p1 + [z] * (nblk - off1 - len(p1))
            b = [z] * off2 + p2 + [z] * (nblk - off2 - len(p2))
            A = []; B = []
            for r in range(nblk):
                if a[r] is z and b[r] is z:
                    A.append(z); B.append(z)
                else:
                    A.append(jnp.where(lo8, a[r], b[r])); B.append(jnp.where(lo8, b[r], a[r]))
            A = pltpu.bitcast(jnp.concatenate(A, 0), bf16)
            B = pltpu.bitcast(jnp.concatenate(B, 0), bf16)
            la = jnp.where(lane_1 < 64, l1, l2); lb = jnp.where(lane_1 < 64, l2, l1)
            r = pltpu.reciprocal(jnp.concatenate([la, lb], 0), full_range=False)
            state["P", u0 // 2] = ((A, r[0:1]), (B, r[1:2]))

        def pv(u):
            j, c, par, e = unit_info(u)
            jb = max(0, j - 2)
            if e == 0:
                exchange(u)
            pf, inv = state["P", u // 2][e]
            if e == 1:
                del state["P", u // 2]
            nk = 128 * (j - jb + 1)
            vt = pltpu.bitcast(vt_u[pl.ds(c * 32 + 16 * e, 16), pl.ds(128 * jb, nk)], bf16)
            o = jnp.dot(vt, pf, preferred_element_type=f32)
            state["o", u] = o * inv

        def fin(u):
            j, c, par, t = unit_info(u)
            if u % 4 != 3:
                return
            os_ = [[state.pop(("o", u - 3 + 2 * pr + e)) for e in range(2)] for pr in range(2)]
            for e in range(2):
                for hh in range(2):
                    acc = None
                    for pr in range(2):
                        piece = os_[pr][e][16 * hh:16 * hh + 16]
                        src = hh if e == 0 else (hh + 2)
                        sh = (32 * (pr - src)) % 128
                        if sh:
                            piece = pltpu.roll(piece, sh, 1)
                        acc = piece if pr == 0 else jnp.where(odd_blk, piece, acc)
                    ot_v[j % 2, pl.ds(64 * c + 32 * e + 16 * hh, 16), :] = acc

        def ocopy(j):
            return pltpu.make_async_copy(out_v.at[pl.ds(j * TQ, TQ), :], out_hbm.at[0, pl.ds(j * TQ, TQ), :], sem_o.at[j])

        def wo_tile(j):
            parts = [ot_v[j % 2, pl.ds(128 * g, 128), :].T.astype(bf16) for g in range(4)]
            o = jnp.concatenate(parts, axis=1)
            a = jnp.dot(o, pltpu.bitcast(wo_u[...], bf16), preferred_element_type=f32)
            for blk, off in enumerate((0, 64, 32, 96)):
                rows = pl.ds(j * TQ + off, 32)
                out_v[rows, :] = (res_v[rows, :] + a[32 * blk:32 * blk + 32]).astype(bf16)
            ocopy(j).start()

        prep_wv()
        layer_norm(0)
        for j in range(NT_):
            if j + 1 < NT_:
                layer_norm(j + 1)
            proj_qk(j)
            proj_vt(j)
        prep_wo()
        ffn()
        NU = NT_ * 32
        for s in range(NU + LB + LW + 1):
            if s < NU:
                qk(s)
            if 0 <= s - LB < NU:
                pv(s - LB)
            if 0 <= s - 4 < NU:
                softmax(s - 4)
            if 0 <= s - LB < NU:
                fin(s - LB)
            w = s - LB - LW
            if 0 <= w < NU and w % 32 == 31:
                wo_tile(w // 32)
        for j in range(NT_):
            ocopy(j).wait()

    return kernel


def build(cfg):
    kernel = make_kernel(cfg)
    scratch = [
        pltpu.VMEM((S, D), bf16),
        pltpu.VMEM((D, 3 * D), bf16),
        pltpu.VMEM((D, D), bf16),
        pltpu.VMEM((D,), bf16),
        pltpu.VMEM((D, F), bf16),
        pltpu.VMEM((D, F), bf16),
        pltpu.VMEM((F, D), bf16),
        pltpu.VMEM((D + 16, D), bf16),
        pltpu.VMEM((D // 2, D), u32),
        pltpu.VMEM((4, S // 2, 128), u32),
        pltpu.VMEM((4, S // 2, 128), u32),
        pltpu.VMEM((D // 2, S), u32),
        pltpu.VMEM((S // 2, D), u32),
        pltpu.VMEM((S, D), f32),
        pltpu.VMEM((2, D, TQ), f32),
        pltpu.VMEM((S, D), bf16),
        pltpu.VMEM((8, 8, 128), u32),
        pltpu.SemaphoreType.DMA((NT_,)),
        pltpu.SemaphoreType.DMA((6,)),
        pltpu.SemaphoreType.DMA((NT_,)),
    ]
    any_spec = pl.BlockSpec(memory_space=pl.ANY)
    flags = cfg.get("flags", {"XLA_TPU_FORCE_LP_LLO_SCHEDULER": True})

    def fn(A_x, A_wqkv, A_wo, B_x, B_w_r, B_w_gate, B_w_up, B_w_down):
        return pl.pallas_call(
            kernel,
            out_shape=jax.ShapeDtypeStruct((1, S, D), bf16),
            in_specs=[any_spec] * 7,
            out_specs=any_spec,
            scratch_shapes=scratch,
            compiler_params=pltpu.CompilerParams(vmem_limit_bytes=100 * 1024 * 1024, flags=flags),
        )(A_x, A_wqkv, A_wo, B_w_r, B_w_gate, B_w_up, B_w_down)
    return jax.jit(fn)


_CFG = {}


def pallas_parallel_sum__sliding_block__moe_arch_mod__prompt_kernel(
    A_x, A_wqkv, A_wo, B_x, B_w_r, B_w_gate, B_w_up, B_w_down,
):
    return build(_CFG)(A_x, A_wqkv, A_wo, B_x, B_w_r, B_w_gate, B_w_up, B_w_down)


pallas_parallel_sum__sliding_block__moe_arch_mod__prompt_kernel = jax.jit(
    pallas_parallel_sum__sliding_block__moe_arch_mod__prompt_kernel)
```

```python
import functools
import math

import jax
import jax.numpy as jnp
from jax import lax
import jax.experimental.pallas as pl
import jax.experimental.pallas.tpu as pltpu

S = 2048
D = 512
H = 32
DH = 16
W = 256
F = 1376
TQ = 128
NT_ = S // TQ
EPS = 1e-5
NEG = -1e9
LOG2E = math.log2(math.e)
QSCALE = (DH ** -0.5) * LOG2E
NT = (((1,), (1,)), ((), ()))
f32 = jnp.float32
bf16 = jnp.bfloat16
u32 = jnp.uint32


def _unpack(u, i):
    return pltpu.unpack_elementwise(u, index=i, packed_dtype=bf16, unpacked_dtype=f32)


def _ipack(a, b):
    return pltpu.pack_elementwise([a, b], packed_dtype=bf16)


def make_kernel(cfg):
    LB = cfg.get("lb", 9)
    LW = cfg.get("lw", 4)

    def kernel(x_hbm, wqkv_hbm, wo_hbm, wr_hbm, wg_hbm, wu_hbm, wd_hbm, out_hbm,
               x_v, wqkv_v, wo_v, wr_v, wg_v, wu_v, wd_v,
               wvt_v, wo_u, q_u, k_u, vt_u, xn_u, res_v, ot_v, out_v, cm_v,
               sem_x, sem_w, sem_o):
        def xcopy(j):
            return pltpu.make_async_copy(x_hbm.at[0, pl.ds(j * TQ, TQ), :], x_v.at[pl.ds(j * TQ, TQ), :], sem_x.at[j])
        cp_wqkv = pltpu.make_async_copy(wqkv_hbm, wqkv_v, sem_w.at[0])
        cp_wr = pltpu.make_async_copy(wr_hbm, wr_v, sem_w.at[1])
        cp_wo = pltpu.make_async_copy(wo_hbm, wo_v, sem_w.at[2])
        cp_wg = pltpu.make_async_copy(wg_hbm, wg_v, sem_w.at[3])
        cp_wu = pltpu.make_async_copy(wu_hbm, wu_v, sem_w.at[4])
        cp_wd = pltpu.make_async_copy(wd_hbm, wd_v, sem_w.at[5])
        xcopy(0).start()
        cp_wr.start()
        cp_wqkv.start()
        for j in range(1, NT_):
            xcopy(j).start()
        cp_wo.start()
        cp_wg.start()
        cp_wu.start()
        cp_wd.start()

        lane8 = lax.broadcasted_iota(jnp.int32, (8, 128), 1)
        for h in range(8):
            cm_v[h] = jnp.where(lane8 // DH == h, u32(0xFFFFFFFF), u32(0))
        lo8 = lane8 < 64
        lane_1 = lax.broadcasted_iota(jnp.int32, (1, 128), 1)
        lane_f = lax.broadcasted_iota(jnp.int32, (16, 128), 1)
        odd_blk = (lane_f // 32) % 2 == 1
        lane32 = lax.broadcasted_iota(jnp.int32, (32, 128), 1)
        row32 = lax.broadcasted_iota(jnp.int32, (32, 128), 0)
        m_old = row32 > (lane32 % 32)

        cp_wr.wait()
        cp_wqkv.wait()

        def prep_wv():
            wv = wqkv_v[:, 2 * D:3 * D]
            wvt = wv.astype(f32).T.astype(bf16)
            u = pltpu.bitcast(wvt, u32)
            e = _unpack(u, 0).reshape(H, 8, D)
            o = _unpack(u, 1).reshape(H, 8, D)
            wpi = jnp.concatenate([e, o], axis=1).reshape(D, D).astype(bf16)
            wvt_v[pl.ds(0, D), :] = wpi
            wr = wr_v[...].reshape(1, D)
            wvt_v[pl.ds(D, 16), :] = jnp.broadcast_to(wr, (16, D))

        def prep_wo():
            cp_wo.wait()
            wo_u[...] = pltpu.bitcast(wo_v[...], u32)

        state = {}

        def layer_norm(j):
            xcopy(j).wait()
            xt = x_v[pl.ds(j * TQ, TQ), :]
            u = pltpu.bitcast(xt, u32)
            halves = []
            for i in range(2):
                xf = _unpack(u, i)
                mean = jnp.mean(xf, axis=-1, keepdims=True)
                xc = xf - mean
                var = jnp.mean(xc * xc, axis=-1, keepdims=True)
                m_b = mean.astype(bf16).astype(f32)
                d_b = (xf - m_b).astype(bf16).astype(f32)
                v_b = (var.astype(bf16) + jnp.asarray(EPS, bf16)).astype(f32)
                sd = jnp.sqrt(v_b).astype(bf16).astype(f32)
                halves.append(d_b / sd)
            xe, xo = halves
            xn_pi = jnp.concatenate([xe, xo], axis=0).astype(bf16)
            un = _ipack(xe, xo)
            xn_u[pl.ds(j * 64, 64), :] = un
            xn_nat = pltpu.bitcast(un, bf16).astype(f32)
            x3 = xn_nat.reshape(8, 16, D)
            xn_sig = pltpu.bitcast(_ipack(x3[:, 0:8, :], x3[:, 8:16, :]).reshape(64, D), bf16)
            res_v[pl.ds(j * TQ, TQ), :] = xt.astype(f32) + xn_nat
            state["xn", j] = (xn_pi, xn_sig)

        def proj_qk(j):
            xn_pi, _ = state["xn", j]
            for part in range(2):
                for g in range(4):
                    c0 = part * D + g * 128
                    r = jnp.dot(xn_pi, wqkv_v[:, c0:c0 + 128], preferred_element_type=f32)
                    if part == 0:
                        r = r * QSCALE
                    pk = _ipack(r[0:64], r[64:128])
                    dst = q_u if part == 0 else k_u
                    dst[g, pl.ds(j * 64, 64), :] = pk

        def proj_vt(j):
            _, xn_sig = state.pop(("xn", j))
            r = lax.dot_general(wvt_v[...], xn_sig, NT, preferred_element_type=f32)
            v3 = r[0:D].reshape(H, 16, 128)
            vt_u[:, pl.ds(j * TQ, TQ)] = _ipack(v3[:, 0:8, :], v3[:, 8:16, :]).reshape(D // 2, 128)
            rr = r[D:D + 8]
            if j == 0:
                state["rmax"] = rr
                state["ridx"] = jnp.zeros((8, 128), jnp.int32)
            else:
                better = rr > state["rmax"]
                state["rmax"] = jnp.where(better, rr, state["rmax"])
                state["ridx"] = jnp.where(better, j, state["ridx"])

        def ffn():
            rmax, rj = state["rmax"], state["ridx"]
            l16 = lane8 % 16
            tok_in = (lane8 // 16) * 16 + (l16 // 2) + 8 * (l16 % 2)
            tok = rj * TQ + tok_in
            best = jnp.max(rmax, axis=1, keepdims=True)
            idx = jnp.min(jnp.where(rmax == best, tok, S))
            idx = jnp.clip(idx, 0, S - 1)
            blk = idx // 16
            cp_wg.wait(); cp_wu.wait(); cp_wd.wait()
            xb = pltpu.bitcast(xn_u[pl.ds(pl.multiple_of(blk * 8, 8), 8), :], bf16)
            g = lax.dot_general(xb, wg_v[...], NT, preferred_element_type=f32).astype(bf16).astype(f32)
            up = lax.dot_general(xb, wu_v[...], NT, preferred_element_type=f32).astype(bf16).astype(f32)
            act = (g * jax.nn.sigmoid(g)).astype(bf16).astype(f32)
            hh = (act * up).astype(bf16)
            y = jnp.dot(hh, wd_v[...], preferred_element_type=f32).astype(bf16).astype(f32)
            gate = jax.nn.sigmoid(best[0:1].astype(bf16).astype(f32)).astype(bf16).astype(f32)
            rows = lax.broadcasted_iota(jnp.int32, (16, D), 0)
            upd = jnp.where(rows == idx % 16, (y * gate).astype(bf16).astype(f32), 0.0)
            sl = pl.ds(pl.multiple_of(blk * 16, 16), 16)
            res_v[sl, :] = res_v[sl, :] + upd

        def unit_info(u):
            b, r = divmod(u, 4)
            j, c = divmod(b, 8)
            par, t = divmod(r, 2)
            return j, c, par, t

        def qk(u):
            j, c, par, t = unit_info(u)
            g, half = c // 2, c % 2
            s = 4 * j + 2 * par + t
            lo = max(0, 32 * s - W)
            hi = 32 * s + 32
            qt = q_u[g, pl.ds(16 * s, 16), :]
            parts = []
            for p in range(4):
                mk = cm_v[4 * half + (p + 2 * t) % 4]
                parts.append(qt & jnp.concatenate([mk, mk], 0))
            b = pltpu.bitcast(jnp.concatenate(parts, axis=0), bf16)
            kk = pltpu.bitcast(k_u[g, pl.ds(lo // 2, (hi - lo) // 2), :], bf16)
            state["s", u] = lax.dot_general(kk, b, NT, preferred_element_type=f32)

        def softmax(u):
            j, c, par, t = unit_info(u)
            s = 4 * j + 2 * par + t
            st = state.pop(("s", u))
            n = st.shape[0]
            lo = max(0, 32 * s - W)
            has_old = 32 * s - W >= 0
            pieces = []
            a = 0
            if has_old:
                pieces.append(jnp.where(m_old, st[0:32], NEG))
                a = 32
            if n - 32 > a:
                pieces.append(st[a:n - 32])
            pieces.append(jnp.where(m_old, NEG, st[n - 32:n]))
            st = jnp.concatenate(pieces, axis=0) if len(pieces) > 1 else pieces[0]
            mx = jnp.max(st, axis=0, keepdims=True)
            p = jnp.exp2(st - mx)
            l = jnp.sum(p, axis=0, keepdims=True)
            p3 = p.reshape(n // 16, 16, 128)
            uu = _ipack(p3[:, 0:8, :], p3[:, 8:16, :])
            state["p", u] = ([uu[r] for r in range(n // 16)], l)

        def exchange(u0):
            j, c, par, _ = unit_info(u0)
            jb = max(0, j - 2)
            nblk = 8 * (j - jb + 1)
            (p1, l1), (p2, l2) = state.pop(("p", u0)), state.pop(("p", u0 + 1))
            z = jnp.zeros((8, 128), u32)
            s0 = 4 * j + 2 * par
            off1 = (max(0, 32 * s0 - W) - 128 * jb) // 16
            off2 = (max(0, 32 * (s0 + 1) - W) - 128 * jb) // 16
            a = [z] * off1 + p1 + [z] * (nblk - off1 - len(p1))
            b = [z] * off2 + p2 + [z] * (nblk - off2 - len(p2))
            A = []; B = []
            for r in range(nblk):
                if a[r] is z and b[r] is z:
                    A.append(z); B.append(z)
                else:
                    A.append(jnp.where(lo8, a[r], b[r])); B.append(jnp.where(lo8, b[r], a[r]))
            A = pltpu.bitcast(jnp.concatenate(A, 0), bf16)
            B = pltpu.bitcast(jnp.concatenate(B, 0), bf16)
            la = jnp.where(lane_1 < 64, l1, l2); lb = jnp.where(lane_1 < 64, l2, l1)
            r = pltpu.reciprocal(jnp.concatenate([la, lb], 0), full_range=False)
            state["P", u0 // 2] = ((A, r[0:1]), (B, r[1:2]))

        def pv(u):
            j, c, par, e = unit_info(u)
            jb = max(0, j - 2)
            if e == 0:
                exchange(u)
            pf, inv = state["P", u // 2][e]
            if e == 1:
                del state["P", u // 2]
            nk = 128 * (j - jb + 1)
            vt = pltpu.bitcast(vt_u[pl.ds(c * 32 + 16 * e, 16), pl.ds(128 * jb, nk)], bf16)
            o = jnp.dot(vt, pf, preferred_element_type=f32)
            state["o", u] = o * inv

        def fin(u):
            j, c, par, t = unit_info(u)
            if u % 4 != 3:
                return
            os_ = [[state.pop(("o", u - 3 + 2 * pr + e)) for e in range(2)] for pr in range(2)]
            for e in range(2):
                for hh in range(2):
                    acc = None
                    for pr in range(2):
                        piece = os_[pr][e][16 * hh:16 * hh + 16]
                        src = hh if e == 0 else (hh + 2)
                        sh = (32 * (pr - src)) % 128
                        if sh:
                            piece = pltpu.roll(piece, sh, 1)
                        acc = piece if pr == 0 else jnp.where(odd_blk, piece, acc)
                    ot_v[j % 2, pl.ds(64 * c + 32 * e + 16 * hh, 16), :] = acc

        def ocopy(j):
            return pltpu.make_async_copy(out_v.at[pl.ds(j * TQ, TQ), :], out_hbm.at[0, pl.ds(j * TQ, TQ), :], sem_o.at[j])

        def wo_tile(j):
            parts = [ot_v[j % 2, pl.ds(128 * g, 128), :].T.astype(bf16) for g in range(4)]
            o = jnp.concatenate(parts, axis=1)
            a = jnp.dot(o, pltpu.bitcast(wo_u[...], bf16), preferred_element_type=f32)
            for blk, off in enumerate((0, 64, 32, 96)):
                rows = pl.ds(j * TQ + off, 32)
                out_v[rows, :] = (res_v[rows, :] + a[32 * blk:32 * blk + 32]).astype(bf16)
            ocopy(j).start()

        prep_wv()
        layer_norm(0)
        for j in range(NT_):
            if j + 1 < NT_:
                layer_norm(j + 1)
            proj_qk(j)
            proj_vt(j)
        prep_wo()
        ffn()
        NU = NT_ * 32
        for s in range(NU + LB + LW + 1):
            if s < NU:
                qk(s)
            if 0 <= s - LB < NU:
                pv(s - LB)
            if 0 <= s - 4 < NU:
                softmax(s - 4)
            if 0 <= s - LB < NU:
                fin(s - LB)
            w = s - LB - LW
            if 0 <= w < NU and w % 32 == 31:
                wo_tile(w // 32)
        for j in range(NT_):
            ocopy(j).wait()

    return kernel


def build(cfg):
    kernel = make_kernel(cfg)
    scratch = [
        pltpu.VMEM((S, D), bf16),
        pltpu.VMEM((D, 3 * D), bf16),
        pltpu.VMEM((D, D), bf16),
        pltpu.VMEM((D,), bf16),
        pltpu.VMEM((F, D), bf16),
        pltpu.VMEM((F, D), bf16),
        pltpu.VMEM((F, D), bf16),
        pltpu.VMEM((D + 16, D), bf16),
        pltpu.VMEM((D // 2, D), u32),
        pltpu.VMEM((4, S // 2, 128), u32),
        pltpu.VMEM((4, S // 2, 128), u32),
        pltpu.VMEM((D // 2, S), u32),
        pltpu.VMEM((S // 2, D), u32),
        pltpu.VMEM((S, D), f32),
        pltpu.VMEM((2, D, TQ), f32),
        pltpu.VMEM((S, D), bf16),
        pltpu.VMEM((8, 8, 128), u32),
        pltpu.SemaphoreType.DMA((NT_,)),
        pltpu.SemaphoreType.DMA((6,)),
        pltpu.SemaphoreType.DMA((NT_,)),
    ]
    any_spec = pl.BlockSpec(memory_space=pltpu.HBM)
    flags = cfg.get("flags", {"XLA_TPU_FORCE_LP_LLO_SCHEDULER": True})

    def fn(A_x, A_wqkv, A_wo, B_x, B_w_r, B_w_gate, B_w_up, B_w_down):
        return pl.pallas_call(
            kernel,
            out_shape=jax.ShapeDtypeStruct((1, S, D), bf16),
            in_specs=[any_spec] * 7,
            out_specs=any_spec,
            scratch_shapes=scratch,
            compiler_params=pltpu.CompilerParams(vmem_limit_bytes=100 * 1024 * 1024, flags=flags),
        )(A_x, A_wqkv, A_wo, B_w_r, B_w_gate.T, B_w_up.T, B_w_down)
    return jax.jit(fn)


_CFG = {}


def pallas_parallel_sum__sliding_block__moe_arch_mod__prompt_kernel(
    A_x, A_wqkv, A_wo, B_x, B_w_r, B_w_gate, B_w_up, B_w_down,
):
    return build(_CFG)(A_x, A_wqkv, A_wo, B_x, B_w_r, B_w_gate, B_w_up, B_w_down)


pallas_parallel_sum__sliding_block__moe_arch_mod__prompt_kernel = jax.jit(
    pallas_parallel_sum__sliding_block__moe_arch_mod__prompt_kernel)
```

```python
import math

import jax
import jax.numpy as jnp
from jax import lax
import jax.experimental.pallas as pl
import jax.experimental.pallas.tpu as pltpu

S = 2048
D = 512
DH = 16
W = 256
F = 1376
TQ = 128
NTILE = S // TQ
EPS = 1e-5
NEG = -1e9
QSCALE = (DH ** -0.5) * math.log2(math.e)
NT = (((1,), (1,)), ((), ()))

XG = (0, 4, 7, NTILE)
QF = 4
LA = 4
LB = 12
LW = 52
NOT = 3

f32 = jnp.float32
bf16 = jnp.bfloat16
u32 = jnp.uint32


def _rb(x):
    return x.astype(bf16).astype(f32)


def _pack(x):
    return pltpu.bitcast(x.astype(bf16), u32)


def _kernel(x_hbm, wqkv_hbm, wo_hbm, wr_hbm, wg_hbm, wu_hbm, wd_hbm, out_hbm,
            x_v, wqk_v, wv_v, wo_v, wr_v, wg_v, wu_v, wd_v,
            wvt_u, wqk_u, wo_u, qb_u, k_u, vt_u, xn_u, res_v, ot_v, out_v, cm_v,
            sem_x, sem_w, sem_o):
    def xcopy(gi):
        rows = pl.ds(XG[gi] * TQ, (XG[gi + 1] - XG[gi]) * TQ)
        return pltpu.make_async_copy(x_hbm.at[0, rows, :], x_v.at[rows, :], sem_x.at[gi])

    def ocopy(j):
        rows = pl.ds(j * TQ, TQ)
        return pltpu.make_async_copy(out_v.at[rows, :], out_hbm.at[0, rows, :], sem_o.at[j])

    cp_wq = pltpu.make_async_copy(wqkv_hbm.at[:, pl.ds(0, D)], wqk_v.at[:, pl.ds(0, D)], sem_w.at[0])
    cp_wk = pltpu.make_async_copy(wqkv_hbm.at[:, pl.ds(D, D)], wqk_v.at[:, pl.ds(D, D)], sem_w.at[7])
    cp_wv = pltpu.make_async_copy(wqkv_hbm.at[:, pl.ds(2 * D, D)], wv_v, sem_w.at[6])
    cp_wr = pltpu.make_async_copy(wr_hbm, wr_v, sem_w.at[1])
    cp_wo = pltpu.make_async_copy(wo_hbm, wo_v, sem_w.at[2])
    cp_wg = pltpu.make_async_copy(wg_hbm, wg_v, sem_w.at[3])
    cp_wu = pltpu.make_async_copy(wu_hbm, wu_v, sem_w.at[4])
    cp_wd = pltpu.make_async_copy(wd_hbm, wd_v, sem_w.at[5])
    late = (cp_wg, cp_wu, cp_wd, cp_wo)
    xcopy(0).start()
    cp_wr.start()
    cp_wq.start()

    lane8 = lax.broadcasted_iota(jnp.int32, (8, 128), 1)
    for h in range(8):
        cm_v[h] = jnp.where(lane8 // DH == h, u32(0xFFFFFFFF), u32(0))
    lo8 = lane8 < 64
    lane1 = lax.broadcasted_iota(jnp.int32, (1, 128), 1)
    lane16 = lax.broadcasted_iota(jnp.int32, (16, 128), 1)
    odd_blk = (lane16 // 32) % 2 == 1
    lane32 = lax.broadcasted_iota(jnp.int32, (32, 128), 1)
    row32 = lax.broadcasted_iota(jnp.int32, (32, 128), 0)
    m_old = row32 > (lane32 % 32)

    cp_wr.wait()
    cp_wk.start()
    xcopy(1).start()
    xcopy(0).wait()
    xcopy(2).start()
    cp_wv.start()
    st = {}
    wr = wr_v[...].astype(f32).reshape(1, D)

    def layer_norm(j):
        if j == XG[2]:
            xcopy(2).wait()
            cp_wv.wait()
        xf = x_v[pl.ds(j * TQ, TQ), :].astype(f32)
        xc = xf - jnp.mean(xf, axis=-1, keepdims=True)
        rstd = lax.rsqrt(jnp.mean(xc * xc, axis=-1, keepdims=True) + EPS)
        xn = (xc * rstd).astype(bf16)
        r = jnp.sum(xc * wr, axis=-1, keepdims=True) * rstd
        xn_u[pl.ds(j * 64, 64), :] = pltpu.bitcast(xn, u32)
        st["xn", j] = xn
        if j == 0:
            st["rmax"] = r
            st["ridx"] = jnp.zeros((TQ, 1), jnp.int32)
        else:
            better = r > st["rmax"]
            st["rmax"] = jnp.where(better, r, st["rmax"])
            st["ridx"] = jnp.where(better, j, st["ridx"])

    ln_next = [0]

    def ln_upto(k):
        while ln_next[0] <= min(k, NTILE - 1):
            layer_norm(ln_next[0])
            ln_next[0] += 1

    def proj_qk(j, parts=(0, 1)):
        xn_val = st.pop(("xn", j), None)
        for part in parts:
            for g in range(4):
                c0 = part * D + g * 128
                if len(parts) == 1:
                    xn = pltpu.bitcast(xn_u[pl.ds(j * 64, 64), :], bf16)
                else:
                    xn = xn_val
                if j == 0:
                    w = wqk_v[:, c0:c0 + 128]
                    wqk_u[:, c0:c0 + 128] = pltpu.bitcast(w, u32)
                else:
                    w = pltpu.bitcast(wqk_u[:, c0:c0 + 128], bf16)
                r = jnp.dot(xn, w, preferred_element_type=f32)
                if part == 1:
                    k_u[g, pl.ds(j * 64, 64), :] = _pack(r)
                    continue
                pk = _pack(r * QSCALE)
                for sub in range(4):
                    qt = pk[16 * sub:16 * sub + 16]
                    for half in range(2):
                        blocks = []
                        for p in range(4):
                            mk = cm_v[4 * half + (p + 2 * (sub % 2)) % 4]
                            blocks.append(qt & jnp.concatenate([mk, mk], 0))
                        qb_u[(4 * j + sub) * 8 + 2 * g + half] = jnp.concatenate(blocks, axis=0)

    def proj_vt(j):
        rows = pl.ds(j * TQ, TQ)
        xn = pltpu.bitcast(xn_u[pl.ds(j * 64, 64), :], bf16)
        for hf in range(2):
            ch = pl.ds(hf * 128, 128)
            w = pltpu.bitcast(wvt_u[ch, :], bf16)
            vt_u[ch, rows] = _pack(lax.dot_general(w, xn, NT, preferred_element_type=f32))
            ffn_step(4)
        res_v[rows, :] = x_v[rows, :].astype(f32) + xn.astype(f32)

    def ffn_select():
        rmax = st["rmax"]
        tok = st["ridx"] * TQ + lax.broadcasted_iota(jnp.int32, (TQ, 1), 0)
        best = jnp.max(rmax, axis=0, keepdims=True)
        idx = jnp.clip(jnp.min(jnp.where(rmax == best, tok, S)), 0, S - 1)
        blk = idx // 16
        st["blk"] = blk
        st["xb"] = pltpu.bitcast(xn_u[pl.ds(pl.multiple_of(blk * 8, 8), 8), :], bf16)
        st["sel"] = lax.broadcasted_iota(jnp.int32, (16, D), 0) == idx % 16
        st["gate"] = _rb(jax.nn.sigmoid(_rb(best)))
        st["zero"] = jnp.minimum(idx, 0)

    def ffn_up(which, f0, f1, kc):
        w = wg_v if which == 0 else wu_v
        r = lax.dot_general(st["xb"][:, kc * 128:(kc + 1) * 128], w[pl.ds(f0, f1 - f0), pl.ds(kc * 128, 128)], NT,
                            preferred_element_type=f32)
        st["gu", which, f0] = r if kc == 0 else st["gu", which, f0] + r

    def ffn_act(f0):
        g = _rb(st.pop(("gu", 0, f0)))
        up = _rb(st.pop(("gu", 1, f0)))
        st["h", f0] = (_rb(g * jax.nn.sigmoid(g)) * up).astype(bf16)

    def ffn_down(f0, f1, nc):
        y = jnp.dot(st["h", f0], wd_v[pl.ds(f0, f1 - f0), pl.ds(nc * 128, 128)], preferred_element_type=f32)
        st["y", nc] = y if f0 == 0 else st["y", nc] + y

    def ffn_finish():
        y = jnp.concatenate([st.pop(("y", nc)) for nc in range(4)], axis=1)
        upd = jnp.where(st["sel"], _rb(_rb(y) * st["gate"]), 0.0)
        rows = pl.ds(pl.multiple_of(st["blk"] * 16, 16), 16)
        res_v[rows, :] = res_v[rows, :] + upd

    chunks = [(a, min(a + 128, F)) for a in range(0, F, 128)]
    ffn_tasks = []
    for i in range(len(chunks) + 1):
        if i < len(chunks):
            ffn_tasks += [(True, ffn_up, (which, *chunks[i], kc)) for kc in range(4) for which in range(2)]
        if i >= 1:
            ffn_tasks.append((False, ffn_act, (chunks[i - 1][0],)))
            ffn_tasks += [(True, ffn_down, (*chunks[i - 1], nc)) for nc in range(4)]
    ffn_tasks.reverse()

    def ffn_step(n):
        for _ in range(n):
            if ffn_tasks:
                _, fn, args = ffn_tasks.pop()
                fn(*args)
                if ffn_tasks and not ffn_tasks[-1][0]:
                    _, fn, args = ffn_tasks.pop()
                    fn(*args)

    def unit(u):
        b, r = divmod(u, 4)
        return (*divmod(b, 8), *divmod(r, 2))

    def qk(u):
        j, c, par, t = unit(u)
        s = 4 * j + 2 * par + t
        lo, hi = max(0, 32 * s - W), 32 * s + 32
        qbd = pltpu.bitcast(qb_u[st["zero"] + (s * 8 + c)], bf16)
        kk = pltpu.bitcast(k_u[c // 2, pl.ds(lo // 2, (hi - lo) // 2), :], bf16)
        st["s", u] = lax.dot_general(kk, qbd, NT, preferred_element_type=f32)

    def softmax(u):
        j, c, par, t = unit(u)
        sc = st.pop(("s", u))
        n = sc.shape[0]
        pieces, a = [], 0
        if 32 * (4 * j + 2 * par + t) - W >= 0:
            pieces.append(jnp.where(m_old, sc[0:32], NEG))
            a = 32
        if n - 32 > a:
            pieces.append(sc[a:n - 32])
        pieces.append(jnp.where(m_old, NEG, sc[n - 32:n]))
        sc = jnp.concatenate(pieces, axis=0) if len(pieces) > 1 else pieces[0]
        p = jnp.exp2(sc - jnp.max(sc, axis=0, keepdims=True))
        st["p", u] = (p, jnp.sum(p, axis=0, keepdims=True))

    def repair(u0):
        j, c, par, _ = unit(u0)
        jb = max(0, j - 2)
        nblk = 16 * (j - jb + 1)
        (p1, l1), (p2, l2) = st.pop(("p", u0)), st.pop(("p", u0 + 1))
        z = jnp.zeros((8, 128), f32)

        def padded(p, s):
            off = (max(0, 32 * s - W) - 128 * jb) // 8
            rows = [p[8 * r:8 * r + 8] for r in range(p.shape[0] // 8)]
            return [z] * off + rows + [z] * (nblk - off - len(rows))

        ta, tb = [], []
        for a, b in zip(padded(p1, 4 * j + 2 * par), padded(p2, 4 * j + 2 * par + 1)):
            empty = a is z and b is z
            ta.append(z if empty else jnp.where(lo8, a, b))
            tb.append(z if empty else jnp.where(lo8, b, a))
        sums = jnp.concatenate([jnp.where(lane1 < 64, l1, l2), jnp.where(lane1 < 64, l2, l1)], 0)
        inv = pltpu.reciprocal(sums, full_range=False)
        st["P", u0 // 2] = ((jnp.concatenate(ta, 0).astype(bf16), inv[0:1]),
                            (jnp.concatenate(tb, 0).astype(bf16), inv[1:2]))

    def pv(u):
        j, c, par, e = unit(u)
        jb = max(0, j - 2)
        if e == 0:
            repair(u)
        pf, inv = st["P", u // 2][e]
        if e == 1:
            del st["P", u // 2]
        vt = pltpu.bitcast(vt_u[pl.ds(c * 32 + 16 * e, 16), pl.ds(128 * jb, 128 * (j - jb + 1))], bf16)
        st["o", u] = jnp.dot(vt, pf, preferred_element_type=f32) * inv

    def gather_heads(u):
        j, c, _, _ = unit(u)
        outs = [[st.pop(("o", u - 3 + 2 * par + e)) for e in range(2)] for par in range(2)]
        for e in range(2):
            for hh in range(2):
                src = hh if e == 0 else hh + 2
                acc = None
                for par in range(2):
                    piece = outs[par][e][16 * hh:16 * hh + 16]
                    shift = (32 * (par - src)) % 128
                    if shift:
                        piece = pltpu.roll(piece, shift, 1)
                    acc = piece if par == 0 else jnp.where(odd_blk, piece, acc)
                ot_v[j % NOT, pl.ds(64 * c + 32 * e + 16 * hh, 16), :] = acc

    def out_proj(j):
        o = jnp.concatenate([ot_v[j % NOT, pl.ds(128 * g, 128), :].T.astype(bf16) for g in range(4)], axis=1)
        a = jnp.dot(o, pltpu.bitcast(wo_u[...], bf16), preferred_element_type=f32)
        for blk, off in enumerate((0, 64, 32, 96)):
            rows = pl.ds(j * TQ + off, 32)
            out_v[rows, :] = (res_v[rows, :] + a[32 * blk:32 * blk + 32]).astype(bf16)
        ocopy(j).start()

    ln_upto(QF - 1)
    cp_wq.wait()
    for j in range(QF):
        proj_qk(j, (0,))
    cp_wk.wait()
    xcopy(1).wait()
    for cp in late:
        cp.start()
    for j in range(QF):
        ln_upto(min(j + QF, XG[2] - 1))
        proj_qk(j, (1,))
    for j in range(QF, NTILE):
        ln_upto(j + 1)
        if j == XG[2]:
            wvt_u[...] = pltpu.bitcast(wv_v[...].astype(f32).T.astype(bf16), u32)
        proj_qk(j)
    for cp in late:
        cp.wait()
    wo_u[...] = pltpu.bitcast(wo_v[...], u32)
    ffn_select()
    for j in range(NTILE):
        proj_vt(j)
    ffn_step(len(ffn_tasks))
    ffn_finish()
    nu = NTILE * 32
    ready = []
    for s in range(nu + LB + LW + 1):
        if s < nu:
            qk(s)
        if 0 <= s - LB < nu:
            pv(s - LB)
        if 0 <= s - LA < nu:
            softmax(s - LA)
        if 0 <= s - LB < nu and (s - LB) % 4 == 3:
            gather_heads(s - LB)
        w = s - LB - LW
        if 0 <= w < nu and w % 32 == 31:
            ready.append(w // 32)
        if ready and (s % 16 == 15 or s >= nu + LB - 1):
            out_proj(ready.pop(0))
    for j in ready:
        out_proj(j)
    for j in range(NTILE):
        ocopy(j).wait()


@jax.jit
def pallas_parallel_sum__sliding_block__moe_arch_mod__prompt_kernel(
    A_x: jax.Array,
    A_wqkv: jax.Array,
    A_wo: jax.Array,
    B_x: jax.Array,
    B_w_r: jax.Array,
    B_w_gate: jax.Array,
    B_w_up: jax.Array,
    B_w_down: jax.Array,
):
    del B_x
    scratch = [
        pltpu.VMEM((S, D), bf16),
        pltpu.VMEM((D, 2 * D), bf16),
        pltpu.VMEM((D, D), bf16),
        pltpu.VMEM((D, D), bf16),
        pltpu.VMEM((D,), bf16),
        pltpu.VMEM((F, D), bf16),
        pltpu.VMEM((F, D), bf16),
        pltpu.VMEM((F, D), bf16),
        pltpu.VMEM((D // 2, D), u32),
        pltpu.VMEM((D // 2, 2 * D), u32),
        pltpu.VMEM((D // 2, D), u32),
        pltpu.VMEM((S // 32 * 8, 64, 128), u32),
        pltpu.VMEM((4, S // 2, 128), u32),
        pltpu.VMEM((D // 2, S), u32),
        pltpu.VMEM((S // 2, D), u32),
        pltpu.VMEM((S, D), f32),
        pltpu.VMEM((NOT, D, TQ), f32),
        pltpu.VMEM((S, D), bf16),
        pltpu.VMEM((8, 8, 128), u32),
        pltpu.SemaphoreType.DMA((3,)),
        pltpu.SemaphoreType.DMA((8,)),
        pltpu.SemaphoreType.DMA((NTILE,)),
    ]
    hbm = pl.BlockSpec(memory_space=pltpu.HBM)
    return pl.pallas_call(
        _kernel,
        out_shape=jax.ShapeDtypeStruct((1, S, D), bf16),
        in_specs=[hbm] * 7,
        out_specs=hbm,
        scratch_shapes=scratch,
        compiler_params=pltpu.CompilerParams(
            vmem_limit_bytes=100 * 1024 * 1024,
            flags={"XLA_TPU_FORCE_LP_LLO_SCHEDULER": True},
        ),
    )(A_x, A_wqkv, A_wo, B_w_r, B_w_gate.T, B_w_up.T, B_w_down)
```
